```python
import os as _os
_os.environ.setdefault("JAX_PLATFORMS", "cpu")
import jax
import jax.numpy as jnp

def _softmax(x, axis=-1):
    return jax.nn.softmax(x, axis=axis)
def _gelu(x):
    return jax.nn.gelu(x, approximate=True)
def _silu(x):
    return jax.nn.silu(x)
def _sigmoid(x):
    return jax.nn.sigmoid(x)
def _layernorm(x, axis=-1, eps=1e-5):
    m = jnp.mean(x, axis=axis, keepdims=True)
    v = jnp.var(x, axis=axis, keepdims=True)
    return (x - m) / jnp.sqrt(v + eps)
def _scatter_add(tgt, idx, src, axis=0):
    return tgt.at[idx].add(src)
def _segment_sum(src, seg, n):
    return jax.ops.segment_sum(src, seg, n)
class _Rng:
    def __init__(self, key):
        self._k = key
    def _next(self):
        self._k, sub = jax.random.split(self._k)
        return sub
    def normal(self, shape):
        return jax.random.normal(self._next(), shape, dtype=jnp.bfloat16)
    def randint(self, lo, hi, shape):
        return jax.random.randint(self._next(), shape, lo, hi, dtype=jnp.int32)
    def uniform(self, shape, lo=0.0, hi=1.0):
        return jax.random.uniform(self._next(), shape, jnp.bfloat16, lo, hi)
    def permutation(self, n):
        return jax.random.permutation(self._next(), n)


kernel_name = 'interleave_layers__linear_attn_block__mha_block__prompt'

def setup_inputs():
    _rng = _Rng(jax.random.key(int.from_bytes(__import__("os").urandom(4), "little")))
    _w = (lambda a: (lambda t: t.astype(jnp.bfloat16) if jnp.issubdtype(t.dtype, jnp.floating) else t)(jnp.asarray(a)))
    def _A_setup():
        B, S, D = 1, 2048, 640
        return {
            "x": _w((lambda *s: _rng.normal(s) * 0.05)(B, S, D)),
            "wqkv": _w((lambda *s: _rng.normal(s) * 0.1)(D, 3 * D)),
            "wo": _w((lambda *s: _rng.normal(s) * 0.05)(D, D)),
        }
    _A_in = _A_setup()

    def _B_setup():
        B, S, D, H = 1, 2048, 640, 32
        return {
            "x": _w((lambda *s: _rng.normal(s) * 0.05)(B, S, D)),
            "wqkv": _w((lambda *s: _rng.normal(s) * 0.1)(D, 3 * D)),
            "wo": _w((lambda *s: _rng.normal(s) * 0.05)(D, D)),
        }
    _B_in = _B_setup()

    return {
        "A_x": _A_in["x"],
        "A_wqkv": _A_in["wqkv"],
        "A_wo": _A_in["wo"],
        "B_x": _B_in["x"],
        "B_wqkv": _B_in["wqkv"],
        "B_wo": _B_in["wo"],
    }

def reference(A_x, A_wqkv, A_wo, B_x, B_wqkv, B_wo):
    def _A_ref(x, wqkv, wo):
        B, S, D = x.shape
        H = 32; Dh = D // H
        qkv = (lambda x, *d: x.transpose(*d))((x @ wqkv).reshape(B, S, 3, H, Dh), 2, 0, 3, 1, 4)
        q, k, v = qkv[0], qkv[1], qkv[2]
        phi = lambda t: jnp.where(t > 0, t + 1, jnp.exp(t)) + 1e-6
        pq, pk = phi(q), phi(k)
        kv = jnp.einsum("bhsd,bhse->bhde", pk, v)
        z = jnp.einsum("bhsd->bhd", pk)
        num = jnp.einsum("bhqd,bhde->bhqe", pq, kv)
        den = jnp.einsum("bhqd,bhd->bhq", pq, z)[..., None] + 1e-6
        o = num / den
        return (lambda x, *d: x.transpose(*d))(o, 0, 2, 1, 3).reshape(B, S, D) @ wo

    def _B_ref(x, wqkv, wo):
        B, S, D = x.shape
        H = 32
        Dh = D // H
        qkv = (lambda x, *d: x.transpose(*d))((x @ wqkv).reshape(B, S, 3, H, Dh), 2, 0, 3, 1, 4)
        q, k, v = qkv[0], qkv[1], qkv[2]
        scores = jnp.einsum("bhqd,bhkd->bhqk", q, k) * (Dh ** -0.5)
        p = _softmax(scores, axis=-1)
        o = jnp.einsum("bhqk,bhkd->bhqd", p, v)
        return (lambda x, *d: x.transpose(*d))(o, 0, 2, 1, 3).reshape(B, S, D) @ wo

    x = A_x
    x = x + _A_ref(_layernorm(x, axis=-1), A_wqkv, A_wo)
    x = x + _B_ref(_layernorm(x, axis=-1), B_wqkv, B_wo)
    x = x + _A_ref(_layernorm(x, axis=-1), A_wqkv, A_wo)
    x = x + _B_ref(_layernorm(x, axis=-1), B_wqkv, B_wo)
    return x
```

```python
import math

import jax
import jax.numpy as jnp
from jax import lax
import jax.experimental.pallas as pl
import jax.experimental.pallas.tpu as pltpu

S, D, H = 2048, 640, 32
DH = D // H
QB = 512
NCG = S // QB
KC = 256
NKC = S // KC
HG = 4
GR = HG * DH
NG = H // HG
NQ = 2
LAG = 2
F32, BF16 = jnp.float32, jnp.bfloat16
QSCALE = math.log2(math.e) / math.sqrt(DH)


def _mm(a, b):
    return lax.dot_general(a, b, (((1,), (0,)), ((), ())), preferred_element_type=F32)


def _mm_nt(a, b):
    return lax.dot_general(a, b, (((1,), (1,)), ((), ())), preferred_element_type=F32)


def _phi(t):
    return jnp.where(t > 0, t + 1.0, jnp.exp(t)) + 1e-6


def _layernorm_t(x):
    m = jnp.mean(x, axis=0, keepdims=True)
    xc = x - m
    v = jnp.mean(xc * xc, axis=0, keepdims=True)
    return (xc * lax.rsqrt(v + 1e-5)).astype(BF16)


def _cols(c):
    return pl.ds(c * QB, QB) if isinstance(c, int) else pl.ds(pl.multiple_of(c * QB, QB), QB)


def _kernel(x_ref, awqkv_ref, awo_ref, bwqkv_ref, bwo_ref, o_ref,
            wa, wb, xt, xn, f0, f1, b0, b1, kp):
    for w_dst, wqkv_ref, wo_ref in ((wa, awqkv_ref, awo_ref), (wb, bwqkv_ref, bwo_ref)):
        for i in range(3):
            w_dst[i * D:(i + 1) * D, :] = wqkv_ref[:, i * D:(i + 1) * D].T
        w_dst[3 * D:, :] = wo_ref[...].T
    for c in range(NCG):
        xc = x_ref[c * QB:(c + 1) * QB, :].T.astype(F32)
        xt[:, _cols(c)] = xc
        xn[:, _cols(c)] = _layernorm_t(xc)

    sub8 = lax.broadcasted_iota(jnp.int32, (8, QB), 0)

    def linear_attention():
        pq, pk = f0, b0
        for c in range(NCG):
            pk[:, _cols(c)] = _phi(_mm(wa[D:2 * D, :], xn[:, _cols(c)])).astype(BF16)
        lhs = jnp.concatenate([xn[...], jnp.ones((16, S), BF16)], axis=0)
        gt = _mm_nt(lhs, pk[...])
        pq[:, _cols(0)] = _phi(_mm(wa[:D, :], xn[:, _cols(0)]))
        kvt = _mm(wa[2 * D:3 * D, :], gt[:D].astype(BF16))
        row_h = lax.broadcasted_iota(jnp.int32, (D, D), 0) // DH
        col_h = lax.broadcasted_iota(jnp.int32, (D, D), 1) // DH
        kvt = jnp.where(row_h == col_h, kvt, 0.0).astype(BF16)
        pq[:, _cols(1)] = _phi(_mm(wa[:D, :], xn[:, _cols(1)]))
        mt = _mm(wa[3 * D:, :], kvt).astype(BF16)
        zsel = jnp.where(
            lax.broadcasted_iota(jnp.int32, (H, D), 0) == lax.broadcasted_iota(jnp.int32, (H, D), 1) // DH,
            jnp.broadcast_to(gt[D:D + 1], (H, D)), 0.0).astype(BF16)
        for c in range(2, NCG):
            pq[:, _cols(c)] = _phi(_mm(wa[:D, :], xn[:, _cols(c)]))
        for c in range(NCG):
            p = pq[:, _cols(c)]
            rden = 1.0 / (_mm(zsel, p.astype(BF16)) + 1e-6)
            parts = []
            for hp in range(H // 2):
                e = jnp.broadcast_to(rden[2 * hp:2 * hp + 1], (8, QB))
                o = jnp.broadcast_to(rden[2 * hp + 1:2 * hp + 2], (8, QB))
                parts += [e, e, jnp.where(sub8 < 4, e, o), o, o]
            pn = (p * jnp.concatenate(parts, axis=0)).astype(BF16)
            xc = xt[:, _cols(c)] + _mm(mt, pn)
            xt[:, _cols(c)] = xc
            xn[:, _cols(c)] = _layernorm_t(xc)

    def head_operands(g, j):
        r32 = lax.broadcasted_iota(jnp.int32, (32, QB), 0)
        qmask = (r32 >= 4 * j) & (r32 < 4 * j + DH)
        q_row = pl.multiple_of(g * GR + 16 * j, 16)
        v_row = pl.multiple_of(g * GR + 40 * (j // 2) + 16 * (j % 2), 8)
        r24 = lax.broadcasted_iota(jnp.int32, (24, KC), 0)
        vmask = (r24 < DH) if j % 2 == 0 else (r24 >= 4)

        def qk(cols, c):
            q = jnp.where(qmask, b1[pl.ds(q_row, 32), cols], jnp.zeros((), BF16))
            rows = pl.ds(c * KC, KC) if isinstance(c, int) else pl.ds(pl.multiple_of(c * KC, KC), KC)
            return _mm(kp[g, rows, :][:, 16 * j:16 * j + 32], q)

        def pv(p, c):
            lanes = pl.ds(c * KC, KC) if isinstance(c, int) else pl.ds(pl.multiple_of(c * KC, KC), KC)
            v = jnp.where(vmask, f1[pl.ds(v_row, 24), lanes], 1.0)
            return _mm(v, p.astype(BF16))

        return qk, pv

    def normalise(acc, j):
        l = acc[20:21] if j % 2 == 0 else acc[0:1]
        return acc * (1.0 / l), l

    def store_group(g, cols, o):
        rows = []
        for e, od in ((o[0], o[1]), (o[2], o[3])):
            rows += [e[:16], jnp.where(sub8 < 4, e[16:], od[:8]), od[8:]]
        b0[pl.ds(pl.multiple_of(g * GR, GR), GR), cols] = jnp.concatenate(rows, axis=0).astype(BF16)

    def softmax_attention():
        kt = f0
        ksum = jnp.zeros((D, 128), F32)
        for c in range(NCG):
            k = _mm(wb[D:2 * D, :], xn[:, _cols(c)])
            kt[:, _cols(c)] = k
            ksum = ksum + ((k[:, :128] + k[:, 128:256]) + (k[:, 256:384] + k[:, 384:]))
        kmean = jnp.sum(ksum, axis=1, keepdims=True) * (1.0 / S)
        for c in range(NCG):
            b1[:, _cols(c)] = (_mm(wb[:D, :], xn[:, _cols(c)]) * QSCALE).astype(BF16)
            kc = (kt[:, _cols(c)] - kmean).astype(BF16)
            for g in range(NG):
                blk = jnp.concatenate([kc[g * GR:(g + 1) * GR], jnp.zeros((128 - GR, QB), BF16)], axis=0)
                kp[g, c * QB:(c + 1) * QB, :] = blk.T
            f1[:, _cols(c)] = _mm(wb[2 * D:3 * D, :], xn[:, _cols(c)])

        def fast(i, bad):
            g = i // (NCG // NQ)
            c0 = (i % (NCG // NQ)) * NQ
            ops = [head_operands(g, j) for j in range(HG)]
            acc, outs, pend = {}, {}, []

            def drain(bad):
                n, j, c, s = pend.pop(0)
                r = ops[j][1](jnp.exp2(s), c)
                acc[n, j] = r if c == 0 else acc[n, j] + r
                if c == NKC - 1:
                    o, l = normalise(acc.pop((n, j)), j)
                    ok = (l >= 1.0) & (l <= 2.0 ** 100)
                    ok = ok & (jnp.max(jnp.where(jnp.abs(o) <= 3e38, 0.0, 1.0), axis=0, keepdims=True) == 0.0)
                    bad = jnp.where(ok, bad, 1.0)
                    outs[n, j] = o
                    if j == HG - 1:
                        store_group(g, _cols(c0 + n), [outs.pop((n, jj)) for jj in range(HG)])
                return bad

            for n in range(NQ):
                for j in range(HG):
                    for c in range(NKC):
                        pend.append((n, j, c, ops[j][0](_cols(c0 + n), c)))
                        if len(pend) > LAG:
                            bad = drain(bad)
            while pend:
                bad = drain(bad)
            return bad

        bad = lax.fori_loop(0, NG * (NCG // NQ), fast, jnp.zeros((1, QB), F32))

        @pl.when(jnp.max(bad) > 0.0)
        def _():
            @pl.loop(0, NG * NCG)
            def _(i):
                g = i // NCG
                cols = _cols(i % NCG)
                outs = []
                for j in range(HG):
                    qk, pv = head_operands(g, j)
                    m = lax.fori_loop(
                        0, NKC, lambda c, m: jnp.maximum(m, jnp.max(qk(cols, c), axis=0, keepdims=True)),
                        jnp.full((1, QB), -jnp.inf, F32))
                    acc = lax.fori_loop(
                        0, NKC, lambda c, a: a + pv(jnp.exp2(qk(cols, c) - m), c), jnp.zeros((24, QB), F32))
                    outs.append(normalise(acc, j)[0])
                store_group(g, cols, outs)

        for c in range(NCG):
            xc = xt[:, _cols(c)] + _mm(wb[3 * D:, :], b0[:, _cols(c)])
            xt[:, _cols(c)] = xc
            xn[:, _cols(c)] = _layernorm_t(xc)

    @pl.loop(0, 2)
    def _(_):
        linear_attention()
        softmax_attention()

    for c in range(NCG):
        o_ref[c * QB:(c + 1) * QB, :] = xt[:, _cols(c)].astype(BF16).T


@jax.jit
def pallas_interleave_layers__linear_attn_block__mha_block__prompt_kernel(
    A_x: jax.Array,
    A_wqkv: jax.Array,
    A_wo: jax.Array,
    B_x: jax.Array,
    B_wqkv: jax.Array,
    B_wo: jax.Array,
):
    del B_x
    out = pl.pallas_call(
        _kernel,
        out_shape=jax.ShapeDtypeStruct((S, D), BF16),
        scratch_shapes=[
            pltpu.VMEM((4 * D, D), BF16),
            pltpu.VMEM((4 * D, D), BF16),
            pltpu.VMEM((D, S), F32),
            pltpu.VMEM((D, S), BF16),
            pltpu.VMEM((D, S), F32),
            pltpu.VMEM((D, S), F32),
            pltpu.VMEM((D, S), BF16),
            pltpu.VMEM((D, S), BF16),
            pltpu.VMEM((NG, S, 128), BF16),
        ],
        compiler_params=pltpu.CompilerParams(vmem_limit_bytes=100 * 2**20),
    )(A_x.reshape(S, D), A_wqkv, A_wo, B_wqkv, B_wo)
    return out.reshape(1, S, D)
```

```python
import math

import jax
import jax.numpy as jnp
from jax import lax
import jax.experimental.pallas as pl
import jax.experimental.pallas.tpu as pltpu

S, D, H = 2048, 640, 32
DH = D // H
QB = 512
NCG = S // QB
KC = 256
NKC = S // KC
HG = 4
GR = HG * DH
NG = H // HG
LAG = 3
F32, BF16, U32 = jnp.float32, jnp.bfloat16, jnp.uint32
QSCALE = math.log2(math.e) / math.sqrt(DH)


def _mm(a, b):
    return lax.dot_general(a, b, (((1,), (0,)), ((), ())), preferred_element_type=F32)


def _mm_nt(a, b):
    return lax.dot_general(a, b, (((1,), (1,)), ((), ())), preferred_element_type=F32)


def _phi(t):
    return jnp.where(t > 0, t + 1.0, jnp.exp(t)) + 1e-6


def _layernorm_t(x):
    m = jnp.mean(x, axis=0, keepdims=True)
    xc = x - m
    v = jnp.mean(xc * xc, axis=0, keepdims=True)
    return (xc * lax.rsqrt(v + 1e-5)).astype(BF16)


def _block(i, size):
    return pl.ds(i * size if isinstance(i, int) else pl.multiple_of(i * size, size), size)


def _cols(c):
    return _block(c, QB)


def _fold_lanes(t):
    return (t[:, :128] + t[:, 128:256]) + (t[:, 256:384] + t[:, 384:])


class _Packed:
    def __init__(self, ref):
        self.ref = ref

    @staticmethod
    def _index(idx):
        if idx is Ellipsis:
            return idx
        *lead, rows, cols = idx
        if isinstance(rows, slice):
            rows = slice(*(None if v is None else v // 2 for v in (rows.start, rows.stop)))
        else:
            start = rows.start // 2
            rows = pl.ds(start if isinstance(start, int) else pl.multiple_of(start, 8), rows.size // 2)
        return (*lead, rows, cols)

    def __getitem__(self, idx):
        return pltpu.bitcast(self.ref[self._index(idx)], BF16)

    def __setitem__(self, idx, val):
        self.ref[self._index(idx)] = pltpu.bitcast(val, U32)


def _kernel(x_hbm, awqkv_hbm, awo_hbm, bwqkv_hbm, bwo_hbm, o_hbm,
            io, rwa, rwoa, rwb, rwob, wa, wb, xt, xn, f0, f1, b0, b1, mt, kp, sems):
    wa, wb, xn, b0, b1, mt, kp = map(_Packed, (wa, wb, xn, b0, b1, mt, kp))

    def x_copy(c):
        rows = pl.ds(c * QB, QB)
        return pltpu.make_async_copy(x_hbm.at[rows], io.at[rows], sems.at[c])

    def wa_copy(i):
        cols = pl.ds(i * D, D)
        return pltpu.make_async_copy(awqkv_hbm.at[:, cols], rwa.at[:, cols], sems.at[NCG + i])

    def out_copy(c):
        rows = pl.ds(c * QB, QB)
        return pltpu.make_async_copy(io.at[rows], o_hbm.at[rows], sems.at[c])

    late_a = [wa_copy(0), wa_copy(2), pltpu.make_async_copy(awo_hbm, rwoa, sems.at[NCG + 3])]
    late_b = [pltpu.make_async_copy(bwqkv_hbm, rwb, sems.at[NCG + 4]),
              pltpu.make_async_copy(bwo_hbm, rwob, sems.at[NCG + 5])]

    sub8 = lax.broadcasted_iota(jnp.int32, (8, QB), 0)
    pq, pk = f0, b0

    def set_x(c, xc):
        xt[:, _cols(c)] = xc
        xn[:, _cols(c)] = _layernorm_t(xc)

    def load_x(c):
        set_x(c, io[c * QB:(c + 1) * QB, :].T.astype(F32))

    def key_features(c):
        p = _phi(_mm(wa[D:2 * D, :], xn[:, _cols(c)]))
        pk[:, _cols(c)] = p.astype(BF16)
        return _fold_lanes(p)

    def gram(c):
        return _mm_nt(pk[:, _cols(c)], xn[:, _cols(c)])

    def linear_attention(zs, gmat, first):
        if first:
            wa[:D, :] = rwa[:, :D].T
            wa[2 * D:, :] = rwa[:, 2 * D:].T
        zrow = jnp.broadcast_to(jnp.sum(zs, axis=1, keepdims=True), (D, 128)).T[:H]
        zsel = jnp.where(
            lax.broadcasted_iota(jnp.int32, (H, D), 0) == lax.broadcasted_iota(jnp.int32, (H, D), 1) // DH,
            zrow, 0.0).astype(BF16)
        same_head = (lax.broadcasted_iota(jnp.int32, (GR, GR), 0) // DH
                     == lax.broadcasted_iota(jnp.int32, (GR, GR), 1) // DH)

        def query_features(c):
            pq[:, _cols(c)] = _phi(_mm(wa[:D, :], xn[:, _cols(c)]))

        def divide_by_den(c):
            p = pq[:, _cols(c)]
            rden = 1.0 / (_mm(zsel, p.astype(BF16)) + 1e-6)
            parts = []
            for hp in range(H // 2):
                e = jnp.broadcast_to(rden[2 * hp:2 * hp + 1], (8, QB))
                o = jnp.broadcast_to(rden[2 * hp + 1:2 * hp + 2], (8, QB))
                parts += [e, e, jnp.where(sub8 < 4, e, o), o, o]
            b1[:, _cols(c)] = (p * jnp.concatenate(parts, axis=0)).astype(BF16)

        query_features(0)
        kv = [jnp.where(same_head, _mm_nt(gmat[g * GR:(g + 1) * GR], wa[2 * D + g * GR:2 * D + (g + 1) * GR, :]),
                        0.0).astype(BF16) for g in range(NG)]
        query_features(1)
        mmat = jnp.concatenate([_mm(kv[g], rwoa[g * GR:(g + 1) * GR, :]).astype(BF16) for g in range(NG)], axis=0)
        divide_by_den(0)
        query_features(2)
        divide_by_den(1)
        mt[...] = mmat.T
        query_features(3)
        divide_by_den(2)
        set_x(0, xt[:, _cols(0)] + _mm(mt[...], b1[:, _cols(0)]))
        divide_by_den(3)
        if first:
            for i in range(3):
                wb[i * D:(i + 1) * D, :] = rwb[:, i * D:(i + 1) * D].T
            wb[3 * D:, :] = rwob[...].T
        for c in range(1, NCG):
            set_x(c, xt[:, _cols(c)] + _mm(mt[...], b1[:, _cols(c)]))

    qt, vt, ot = b0, f1, b1

    def head_operands(g, j):
        r32 = lax.broadcasted_iota(jnp.int32, (32, QB), 0)
        qmask = (r32 >= 4 * j) & (r32 < 4 * j + DH)
        q_row = pl.multiple_of(g * GR + 16 * j, 16)
        v_row = pl.multiple_of(g * GR + 40 * (j // 2) + 16 * (j % 2), 8)
        r24 = lax.broadcasted_iota(jnp.int32, (24, KC), 0)
        vmask = (r24 < DH) if j % 2 == 0 else (r24 >= 4)

        def qk(cols, c):
            q = jnp.where(qmask, qt[pl.ds(q_row, 32), cols], jnp.zeros((), BF16))
            return _mm(kp[g, _block(c, KC), :][:, 16 * j:16 * j + 32], q)

        def pv(p, c):
            v = jnp.where(vmask, vt[pl.ds(v_row, 24), _block(c, KC)], 1.0)
            return _mm(v, p.astype(BF16))

        return qk, pv

    def normalise(acc, j):
        l = acc[20:21] if j % 2 == 0 else acc[0:1]
        return acc * (1.0 / l), l

    def store_group(g, cols, o):
        rows = []
        for e, od in ((o[0], o[1]), (o[2], o[3])):
            rows += [e[:16], jnp.where(sub8 < 4, e[16:], od[:8]), od[8:]]
        ot[_block(g, GR), cols] = jnp.concatenate(rows, axis=0).astype(BF16)

    def softmax_attention():
        kt = f0
        ksum = jnp.zeros((D, 128), F32)
        for c in range(NCG):
            k = _mm(wb[D:2 * D, :], xn[:, _cols(c)])
            kt[:, _cols(c)] = k
            ksum = ksum + _fold_lanes(k)
        kmean = jnp.sum(ksum, axis=1, keepdims=True) * (1.0 / S)
        for c in range(NCG):
            qt[:, _cols(c)] = (_mm(wb[:D, :], xn[:, _cols(c)]) * QSCALE).astype(BF16)
            kc = (kt[:, _cols(c)] - kmean).astype(BF16)
            for g in range(NG):
                blk = jnp.concatenate([kc[g * GR:(g + 1) * GR], jnp.zeros((128 - GR, QB), BF16)], axis=0)
                kp[g, c * QB:(c + 1) * QB, :] = blk.T
            vt[:, _cols(c)] = _mm(wb[2 * D:3 * D, :], xn[:, _cols(c)])

        def fast(g, bad):
            ops = [head_operands(g, j) for j in range(HG)]
            acc, outs, pend = {}, {}, []

            def drain(bad):
                n, j, c, s = pend.pop(0)
                r = ops[j][1](jnp.exp2(s), c)
                acc[n, j] = r if c == 0 else acc[n, j] + r
                if c == NKC - 1:
                    o, l = normalise(acc.pop((n, j)), j)
                    ok = (l >= 1.0) & (l <= 2.0 ** 100)
                    ok = ok & (jnp.max(jnp.where(jnp.abs(o) <= 3e38, 0.0, 1.0), axis=0, keepdims=True) == 0.0)
                    bad = jnp.where(ok, bad, 1.0)
                    outs[n, j] = o
                    if j == HG - 1:
                        store_group(g, _cols(n), [outs.pop((n, jj)) for jj in range(HG)])
                return bad

            for n in range(NCG):
                for j in range(HG):
                    for c in range(NKC):
                        pend.append((n, j, c, ops[j][0](_cols(n), c)))
                        if len(pend) > LAG:
                            bad = drain(bad)
            while pend:
                bad = drain(bad)
            return bad

        bad = lax.fori_loop(0, NG, fast, jnp.zeros((1, QB), F32))

        @pl.when(jnp.max(bad) > 0.0)
        def _():
            @pl.loop(0, NG * NCG)
            def _(i):
                g = i // NCG
                cols = _cols(i % NCG)
                outs = []
                for j in range(HG):
                    qk, pv = head_operands(g, j)
                    m = lax.fori_loop(
                        0, NKC, lambda c, m: jnp.maximum(m, jnp.max(qk(cols, c), axis=0, keepdims=True)),
                        jnp.full((1, QB), -jnp.inf, F32))
                    acc = lax.fori_loop(
                        0, NKC, lambda c, a: a + pv(jnp.exp2(qk(cols, c) - m), c), jnp.zeros((24, QB), F32))
                    outs.append(normalise(acc, j)[0])
                store_group(g, cols, outs)

    def after_softmax(c):
        return xt[:, _cols(c)] + _mm(wb[3 * D:, :], ot[:, _cols(c)])

    x_copy(0).start()
    wa_copy(1).start()
    x_copy(0).wait()
    x_copy(1).start()
    load_x(0)
    wa_copy(1).wait()
    x_copy(2).start()
    x_copy(3).start()
    wa[D:2 * D, :] = rwa[:, D:2 * D].T
    zs = key_features(0)
    x_copy(1).wait()
    for cp in late_a:
        cp.start()
    gm = gram(0)
    load_x(1)
    zs = zs + key_features(1)
    x_copy(2).wait()
    x_copy(3).wait()
    for cp in late_b:
        cp.start()
    gm = gm + gram(1)
    load_x(2)
    load_x(3)
    zs = zs + key_features(2)
    zs = zs + key_features(3)
    gm = gm + gram(2)
    gm = gm + gram(3)
    for cp in late_a + late_b:
        cp.wait()
    linear_attention(zs, gm.astype(BF16), True)

    softmax_attention()
    set_x(0, after_softmax(0))
    set_x(1, after_softmax(1))
    zs = key_features(0)
    set_x(2, after_softmax(2))
    zs = zs + key_features(1)
    set_x(3, after_softmax(3))
    zs = zs + key_features(2)
    gm = gram(0)
    zs = zs + key_features(3)
    for c in range(1, NCG):
        gm = gm + gram(c)
    linear_attention(zs, gm.astype(BF16), False)

    softmax_attention()
    for c in range(NCG):
        io[c * QB:(c + 1) * QB, :] = after_softmax(c).astype(BF16).T
        out_copy(c).start()
    for c in range(NCG):
        out_copy(c).wait()


@jax.jit
def pallas_interleave_layers__linear_attn_block__mha_block__prompt_kernel(
    A_x: jax.Array,
    A_wqkv: jax.Array,
    A_wo: jax.Array,
    B_x: jax.Array,
    B_wqkv: jax.Array,
    B_wo: jax.Array,
):
    del B_x
    out = pl.pallas_call(
        _kernel,
        out_shape=jax.ShapeDtypeStruct((S, D), BF16),
        in_specs=[pl.BlockSpec(memory_space=pl.ANY)] * 5,
        out_specs=pl.BlockSpec(memory_space=pl.ANY),
        scratch_shapes=[
            pltpu.VMEM((S, D), BF16),
            pltpu.VMEM((D, 3 * D), BF16),
            pltpu.VMEM((D, D), BF16),
            pltpu.VMEM((D, 3 * D), BF16),
            pltpu.VMEM((D, D), BF16),
            pltpu.VMEM((3 * D // 2, D), U32),
            pltpu.VMEM((4 * D // 2, D), U32),
            pltpu.VMEM((D, S), F32),
            pltpu.VMEM((D // 2, S), U32),
            pltpu.VMEM((D, S), F32),
            pltpu.VMEM((D, S), F32),
            pltpu.VMEM((D // 2, S), U32),
            pltpu.VMEM((D // 2, S), U32),
            pltpu.VMEM((D // 2, D), U32),
            pltpu.VMEM((NG, S // 2, 128), U32),
            pltpu.SemaphoreType.DMA((NCG + 6,)),
        ],
        compiler_params=pltpu.CompilerParams(vmem_limit_bytes=100 * 2**20),
    )(A_x.reshape(S, D), A_wqkv, A_wo, B_wqkv, B_wo)
    return out.reshape(1, S, D)
```
